```python
import os as _os
_os.environ.setdefault("JAX_PLATFORMS", "cpu")
import jax
import jax.numpy as jnp

def _softmax(x, axis=-1):
    return jax.nn.softmax(x, axis=axis)
def _gelu(x):
    return jax.nn.gelu(x, approximate=True)
def _silu(x):
    return jax.nn.silu(x)
def _sigmoid(x):
    return jax.nn.sigmoid(x)
def _layernorm(x, axis=-1, eps=1e-5):
    m = jnp.mean(x, axis=axis, keepdims=True)
    v = jnp.var(x, axis=axis, keepdims=True)
    return (x - m) / jnp.sqrt(v + eps)
def _scatter_add(tgt, idx, src, axis=0):
    return tgt.at[idx].add(src)
def _segment_sum(src, seg, n):
    return jax.ops.segment_sum(src, seg, n)
class _Rng:
    def __init__(self, key):
        self._k = key
    def _next(self):
        self._k, sub = jax.random.split(self._k)
        return sub
    def normal(self, shape):
        return jax.random.normal(self._next(), shape, dtype=jnp.bfloat16)
    def randint(self, lo, hi, shape):
        return jax.random.randint(self._next(), shape, lo, hi, dtype=jnp.int32)
    def uniform(self, shape, lo=0.0, hi=1.0):
        return jax.random.uniform(self._next(), shape, jnp.bfloat16, lo, hi)
    def permutation(self, n):
        return jax.random.permutation(self._next(), n)


kernel_name = 'recurrent_scan__sliding_block__dense_activation_mish__prompt'

def setup_inputs():
    _rng = _Rng(jax.random.key(int.from_bytes(__import__("os").urandom(4), "little")))
    _w = (lambda a: (lambda t: t.astype(jnp.bfloat16) if jnp.issubdtype(t.dtype, jnp.floating) else t)(jnp.asarray(a)))
    def _A_setup():
        B, S, D = 1, 2048, 576
        return {
            "x": _w((lambda *s: _rng.normal(s) * 0.05)(B, S, D)),
            "wqkv": _w((lambda *s: _rng.normal(s) * 0.1)(D, 3 * D)),
            "wo": _w((lambda *s: _rng.normal(s) * 0.1)(D, D)),
        }
    _A_in = _A_setup()

    def _B_setup():
        B, S, D, F = 1, 2048, 576, 4608
        return {
            "x": _w((lambda *s: _rng.normal(s) * 0.05)(B, S, D)),
            "w1": _w((lambda *s: _rng.normal(s) * 0.05)(D, F) * (D ** -0.5)),
            "b1": _w((lambda *s: _rng.normal(s) * 0.05)(F)),
            "w2": _w((lambda *s: _rng.normal(s) * 0.05)(F, D) * (F ** -0.5)),
        }
    _B_in = _B_setup()

    return {
        "A_x": _A_in["x"],
        "A_wqkv": _A_in["wqkv"],
        "A_wo": _A_in["wo"],
        "B_x": _B_in["x"],
        "B_w1": _B_in["w1"],
        "B_b1": _B_in["b1"],
        "B_w2": _B_in["w2"],
    }

def reference(A_x, A_wqkv, A_wo, B_x, B_w1, B_b1, B_w2):
    def _A_ref(x, wqkv, wo):
        B, S, D = x.shape
        H = 32; Dh = D // H; W = 256
        qkv = (lambda x, *d: x.transpose(*d))((x @ wqkv).reshape(B, S, 3, H, Dh), 2, 0, 3, 1, 4)
        q, k, v = qkv[0], qkv[1], qkv[2]
        scores = jnp.einsum("bhqd,bhkd->bhqk", q, k) * (Dh ** -0.5)
        idx = jnp.arange(S)
        mask = (idx[:, None] - idx[None, :] >= 0) & (idx[:, None] - idx[None, :] < W)
        scores = jnp.where(mask[None, None], scores, -1e9)
        p = _softmax(scores, axis=-1)
        o = jnp.einsum("bhqk,bhkd->bhqd", p, v)
        return (lambda x, *d: x.transpose(*d))(o, 0, 2, 1, 3).reshape(B, S, D) @ wo

    def _B_ref(x, w1, b1, w2):
        h = jnp.einsum("bsd,df->bsf", x, w1) + b1
        sp = jnp.log1p(jnp.exp(-jnp.abs(h))) + jnp.where(h > 0, h, jnp.zeros_like(h))
        act = h * jnp.tanh(sp)
        return jnp.einsum("bsf,fd->bsd", act, w2)

    x = A_x
    xn = _layernorm(x, axis=-1)
    s = _A_ref(xn, A_wqkv, A_wo)
    g = _silu(_B_ref(xn, B_w1, B_b1, B_w2))
    return x + s * g
```

```python
import functools
import jax
import jax.numpy as jnp
import numpy as np
from jax import lax
import jax.experimental.pallas as pl
import jax.experimental.pallas.tpu as pltpu

S, D, F, H, DH, W = 2048, 576, 4608, 32, 18, 256
T = 256
FC = 256
SH = 2
NT = (((1,), (1,)), ((), ()))
NS = S // T
NB = T // 128
f32, bf16 = jnp.float32, jnp.bfloat16
KW = [min(72 * g // 16 * 16, D - 128) for g in range(8)]
LOG2E = 1.4426950408889634


def _kernel(x_hbm, wqkv_hbm, wo_hbm, b1_ref, w1_hbm, w2_hbm, o_ref,
            wqkv_ref, wo_ref, w1_v, w2_v, wT, xn_scr, qT_scr, k_scr, vT_scr, oT_scr, x_scr, xnT_scr, sems, xsems):
    i = pl.program_id(0)
    cp1 = pltpu.make_async_copy(w1_hbm, w1_v, sems.at[0])
    cp2 = pltpu.make_async_copy(w2_hbm, w2_v, sems.at[1])
    RC = [(0, 128), (128, 128), (256, 128), (384, 192)]
    cq = [pltpu.make_async_copy(wqkv_hbm.at[r:r + n], wqkv_ref.at[r:r + n], sems.at[3 + j]) for j, (r, n) in enumerate(RC)]
    co = pltpu.make_async_copy(wo_hbm, wo_ref, sems.at[2])

    def cx(j):
        return pltpu.make_async_copy(x_hbm.at[:, pl.ds(pl.multiple_of(j * T, T), T)], x_scr.at[j], xsems.at[j])

    def ln(j, slot):
        x = x_scr[j].astype(f32)
        mu = jnp.mean(x, axis=0, keepdims=True)
        xc = x - mu
        var = jnp.mean(xc * xc, axis=0, keepdims=True)
        xnT = (xc * lax.rsqrt(var + 1e-5)).astype(bf16)
        xnT_scr[slot] = xnT
        xn_scr[j] = xnT.T

    @pl.when(i == 0)
    def _():
        cx(0).start()
        for c in cq:
            c.start()
        cx(1).start()

    @pl.when(i == 0)
    def _():
        k_scr[:, 0:W, :] = jnp.zeros((8, W, 128), bf16)
        vT_scr[0:2] = jnp.zeros((2, D, 128), bf16)
        cx(0).wait()
        ln(0, 0)
        for c, (r, n) in zip(cq, RC):
            c.wait()
            wT[:, r:r + n] = wqkv_ref[r:r + n, :].T
        for j in range(2, NS):
            cx(j).start()
        co.start()
        cp1.start()
        cp2.start()

    @pl.when(i < NS - 1)
    def _():
        cx(i + 1).wait()

    @pl.when(i < NS)
    def _():
        xnT = xnT_scr[i % 2]
        ln(jnp.minimum(i + 1, NS - 1), (i + 1) % 2)
        qkv = jnp.dot(wT[...], xnT, preferred_element_type=f32)
        qT_scr[i] = (qkv[0:D] * (DH ** -0.5 * LOG2E)).astype(bf16)
        kT = qkv[D:2 * D].astype(bf16)
        r = pl.multiple_of(W + i * T, T)
        for g in range(8):
            k_scr[g, pl.ds(r, T), :] = kT[KW[g]:KW[g] + 128].T
        vT = qkv[2 * D:3 * D].astype(bf16)
        for jb in range(NB):
            vT_scr[2 + i * NB + jb] = vT[:, 128 * jb:128 * jb + 128]

    @pl.when(i == NS)
    def _():
        co.wait()
        cp1.wait()
        cp2.wait()

    @pl.when(i >= NS)
    def _():
        _main(i - NS, x_scr, b1_ref, o_ref, w1_v, w2_v, wo_ref, xn_scr, qT_scr, k_scr, vT_scr, oT_scr)


def _main(i, x_ref, b1_ref, o_ref, w1_v, w2_v, woT, xn_scr, qT_scr, k_scr, vT_scr, oT_scr):
    xn = xn_scr[i]
    qT = qT_scr[i]
    u32 = jnp.uint32
    kl = lax.broadcasted_iota(jnp.int32, (32, 128), 0)
    ql = lax.broadcasted_iota(jnp.int32, (32, 128), 1)
    tri = kl <= (ql & 31)
    trib = pltpu.bitcast(jnp.where(tri, 1.0, 0.0).astype(bf16), u32)
    trib = (trib >> 7 & 0x00010001) * 0xFFFF
    r32 = kl
    NEG = -1e30
    qTp = pltpu.bitcast(qT, u32)
    b1 = b1_ref[...].astype(f32).reshape(1, F)

    def odd(n, bit):
        return (lax.broadcasted_iota(jnp.int32, (n, 128), 1) & bit) != 0

    def scores(g, jb):
        r0 = 72 * g // 16 * 16
        slab = qTp[r0 // 2:r0 // 2 + 40, 128 * jb:128 * jb + 128]
        row = 2 * lax.broadcasted_iota(jnp.int32, (40, 128), 0) + (r0 - 72 * g)
        qa = lax.broadcasted_iota(jnp.int32, (40, 128), 1) >> 5
        diag = (row >= DH * qa) & (row < DH * qa + DH)
        R = [slab] + [pltpu.roll(slab, 32 * s_, 1) for s_ in range(1, 4)]
        out = []
        for b in range(4):
            t = R[-b % 4]
            for a in range(1, 4):
                t = jnp.where(qa == a, R[(a - b) % 4], t)
            t = pltpu.bitcast(jnp.where(diag, t, u32(0)), bf16)
            qm = jnp.concatenate([jnp.zeros((128, 128), bf16), t, jnp.zeros((128, 128), bf16)], axis=0)[128 + KW[g] - r0:256 + KW[g] - r0]
            kw = k_scr[g, pl.ds(pl.multiple_of(i * T + 128 * jb + 32 * b, 32), 288), :]
            out.append(jnp.dot(kw, qm, preferred_element_type=f32))
        return out

    def prob(sT, jb, b):
        s_f = sT[0:32]
        s_c = sT[32:256]
        if jb < 2:
            n = 256 - 128 * jb - 32 * b
            pen = jnp.where(i > 0, 0.0, NEG).astype(f32)
            s_f = s_f + pen
            if n > 32:
                s_c = jnp.concatenate([s_c[:n - 32] + pen] + ([s_c[n - 32:]] if n < 256 else []), axis=0)
        s_m = jnp.where(tri, sT[256:288], s_f)
        sc = jnp.concatenate([s_m, s_c], axis=0)
        m = jnp.max(sc, axis=0, keepdims=True)
        p = jnp.exp2(sc - m)
        l = jnp.sum(p, axis=0, keepdims=True)
        pb = pltpu.bitcast(p.astype(bf16), u32)
        pd = pb[0:16] & trib
        z = [jnp.zeros((16, 128), u32)]
        return jnp.concatenate(z * b + [pb[0:16] ^ pd, pb[16:], pd] + z * (3 - b), axis=0), jnp.broadcast_to(pl.reciprocal(l, approx=True), (8, 128))

    def blk_t(t):
        for st in (1, 2):
            o = odd(t[0].shape[0], 32 * st)
            n = list(t)
            for u in range(4):
                if not u & st:
                    n[u] = jnp.where(o, pltpu.roll(t[u + st], 32 * st, 1), t[u])
                    n[u + st] = jnp.where(o, t[u + st], pltpu.roll(t[u], 128 - 32 * st, 1))
            t = n
        return t

    def probs(sts, jb):
        r = [prob(sT, jb, b) for b, sT in enumerate(sts)]
        return [(pltpu.bitcast(p, bf16), l[0:1]) for p, l in zip(blk_t([x[0] for x in r]), blk_t([x[1] for x in r]))]

    def pv(h, jb, pT, rl):
        f0 = DH * h
        r0 = (f0 // 16) * 16
        vw = jnp.concatenate([vT_scr[i * NB + jb + u, r0:r0 + 32, :] for u in range(3)], axis=1)
        oh = jnp.dot(vw, pT, preferred_element_type=f32) * rl
        lo = (f0 // 8) * 8
        hi = ((f0 + DH + 7) // 8) * 8
        oh = oh[lo - r0:hi - r0]
        if lo != f0:
            old = oT_scr[lo:lo + 8, 128 * jb:128 * jb + 128]
            oh = jnp.concatenate([jnp.where(r32[0:8] >= f0 - lo, oh[0:8], old), oh[8:]], axis=0)
        oT_scr[lo:hi, 128 * jb:128 * jb + 128] = oh

    y = jnp.zeros((D, T), f32)
    NC = F // FC

    def ffn1(c):
        return jnp.dot(xn, w1_v[:, c * FC:(c + 1) * FC], preferred_element_type=f32) + b1[:, c * FC:(c + 1) * FC]

    def mish(hh):
        e = jnp.exp(jnp.minimum(hh, 20.0))
        n = e * (e + 2.0)
        return (hh * n * pl.reciprocal(n + 2.0, approx=True)).astype(bf16)

    units = [(h, jb) for h in range(8) for jb in range(NB)]
    cuts = [min(len(units), max(0, round((c - SH) * len(units) / (NC - SH)))) for c in range(NC + 1)]
    hh = ffn1(0)
    prev = []
    cuts.append(cuts[-1])
    sn = [scores(h, jb) for h, jb in units[cuts[0]:cuts[1]]]
    for c in range(NC):
        hs = units[cuts[c]:cuts[c + 1]]
        ss = sn
        ss = [scores(h, jb) for h, jb in hs]
        act = mish(hh)
        y = y + lax.dot_general(w2_v[:, c * FC:(c + 1) * FC], act, NT, preferred_element_type=f32)
        ps = [probs(s_, jb) for s_, (h, jb) in zip(ss, hs)]
        hn = ffn1(c + 1) if c + 1 < NC else None
        [pv(4 * g + a, jb, pT, rl) for (g, jb), pp in zip(hs, ps) for a, (pT, rl) in enumerate(pp)]
        hh = hn
        prev = list(zip(hs, ps))
    g = y * pl.reciprocal(1.0 + jnp.exp(-y), approx=True)
    sT_ = lax.dot_general(woT[...], oT_scr[...].astype(bf16), (((0,), (0,)), ((), ())), preferred_element_type=f32)
    o_ref[...] = (x_ref[i].astype(f32) + sT_ * g).astype(o_ref.dtype)


@jax.jit
def pallas_recurrent_scan__sliding_block__dense_activation_mish__prompt_kernel(A_x, A_wqkv, A_wo, B_x, B_w1, B_b1, B_w2):
    bf16 = jnp.bfloat16
    HB = pl.BlockSpec(memory_space=pltpu.MemorySpace.HBM)
    x = A_x.reshape(S, D).T
    out = pl.pallas_call(
        _kernel,
        grid=(2 * NS,),
        in_specs=[
            HB,
            HB,
            HB,
            pl.BlockSpec((F,), lambda i: (0,)),
            HB,
            HB,
        ],
        out_specs=pl.BlockSpec((D, T), lambda i: (0, jnp.maximum(i - NS, 0))),
        out_shape=jax.ShapeDtypeStruct((D, S), A_x.dtype),
        scratch_shapes=[
            pltpu.VMEM((D, 3 * D), bf16), pltpu.VMEM((D, D), bf16), pltpu.VMEM((D, F), bf16), pltpu.VMEM((D, F), bf16),
            pltpu.VMEM((3 * D, D), bf16),
            pltpu.VMEM((NS, T, D), bf16), pltpu.VMEM((NS, D, T), bf16),
            pltpu.VMEM((8, W + S, 128), bf16), pltpu.VMEM((2 + S // 128, D, 128), bf16),
            pltpu.VMEM((D, T), jnp.float32),
            pltpu.VMEM((NS, D, T), bf16), pltpu.VMEM((2, D, T), bf16),
            pltpu.SemaphoreType.DMA((7,)), pltpu.SemaphoreType.DMA((NS,)),
        ],
        compiler_params=pltpu.CompilerParams(dimension_semantics=("arbitrary",), vmem_limit_bytes=100 * 1024 * 1024),
    )(x, A_wqkv, A_wo, B_b1, B_w1, B_w2.T)
    return out.T.reshape(1, S, D)
```
